```python
import os as _os
_os.environ.setdefault("JAX_PLATFORMS", "cpu")
import jax
import jax.numpy as jnp

def _softmax(x, axis=-1):
    return jax.nn.softmax(x, axis=axis)
def _gelu(x):
    return jax.nn.gelu(x, approximate=True)
def _silu(x):
    return jax.nn.silu(x)
def _sigmoid(x):
    return jax.nn.sigmoid(x)
def _layernorm(x, axis=-1, eps=1e-5):
    m = jnp.mean(x, axis=axis, keepdims=True)
    v = jnp.var(x, axis=axis, keepdims=True)
    return (x - m) / jnp.sqrt(v + eps)
def _scatter_add(tgt, idx, src, axis=0):
    return tgt.at[idx].add(src)
def _segment_sum(src, seg, n):
    return jax.ops.segment_sum(src, seg, n)
class _Rng:
    def __init__(self, key):
        self._k = key
    def _next(self):
        self._k, sub = jax.random.split(self._k)
        return sub
    def normal(self, shape):
        return jax.random.normal(self._next(), shape, dtype=jnp.bfloat16)
    def randint(self, lo, hi, shape):
        return jax.random.randint(self._next(), shape, lo, hi, dtype=jnp.int32)
    def uniform(self, shape, lo=0.0, hi=1.0):
        return jax.random.uniform(self._next(), shape, jnp.bfloat16, lo, hi)
    def permutation(self, n):
        return jax.random.permutation(self._next(), n)


kernel_name = 'standalone__gqa_block_cached__near_ridge'

def setup_inputs():
    _rng = _Rng(jax.random.key(int.from_bytes(__import__("os").urandom(4), "little")))
    _w = (lambda a: (lambda t: t.astype(jnp.bfloat16) if jnp.issubdtype(t.dtype, jnp.floating) else t)(jnp.asarray(a)))
    B, Sq, D = 16, 128, 576
    Hq, Hkv, Sk, Dh = 32, 16, 1024, 128
    assert Hq % Hkv == 0, (Hq, Hkv)
    return {
        "x": _w((lambda *s: _rng.normal(s) * 0.8)(B, Sq, D)),
        "k_cache": _w((lambda *s: _rng.normal(s) * 0.8)(B, Hkv, Sk, Dh)),
        "v_cache": _w((lambda *s: _rng.normal(s) * 0.05)(B, Hkv, Sk, Dh)),
        "wq": _w((lambda *s: _rng.normal(s) * 0.8)(D, Hq * Dh) * (D ** -0.5)),
        "wo": _w((lambda *s: _rng.normal(s) * 0.05)(Hq * Dh, D) * ((Hq * Dh) ** -0.5)),
    }

def reference(x, k_cache, v_cache, wq, wo):
    B, Sq, D = x.shape
    Hq, Dh = 32, 128
    Hkv = k_cache.shape[1]
    rep = Hq // Hkv
    q = (lambda x, *d: x.transpose(*d))((x @ wq).reshape(B, Sq, Hq, Dh), 0, 2, 1, 3)
    k = jnp.repeat(k_cache, rep, axis=1)
    v = jnp.repeat(v_cache, rep, axis=1)
    scores = jnp.einsum("bhqd,bhkd->bhqk", q, k) * (Dh ** -0.5)
    p = _softmax(scores, axis=-1)
    o = jnp.einsum("bhqk,bhkd->bhqd", p, v)
    return (lambda x, *d: x.transpose(*d))(o, 0, 2, 1, 3).reshape(B, Sq, Hq * Dh) @ wo
```

```python
import functools

import jax
import jax.numpy as jnp
import jax.experimental.pallas as pl
import jax.experimental.pallas.tpu as pltpu


def _gqa_kernel(x_ref, k_ref, v_ref, wq_ref, wo_ref, o_ref, acc_ref, *, hb, rep, dh, scale):
    g = pl.program_id(1)
    sq = x_ref.shape[1]
    gw = rep * dh

    @pl.when(g == 0)
    def _():
        acc_ref[...] = jnp.zeros(acc_ref.shape, acc_ref.dtype)

    x = x_ref[0]
    for j in range(hb):
        col = pl.multiple_of((g * hb + j) * gw, gw)
        q = jnp.dot(x, wq_ref[:, pl.ds(col, gw)], preferred_element_type=jnp.float32)
        q = q.astype(jnp.bfloat16)
        q2 = jnp.concatenate([q[:, r * dh:(r + 1) * dh] for r in range(rep)], axis=0)
        s = jax.lax.dot_general(q2, k_ref[0, j], (((1,), (1,)), ((), ())),
                                preferred_element_type=jnp.float32) * scale
        m = jnp.max(s, axis=-1, keepdims=True)
        p = jnp.exp(s - m)
        l = jnp.sum(p, axis=-1, keepdims=True)
        o = jnp.dot(p.astype(jnp.bfloat16), v_ref[0, j], preferred_element_type=jnp.float32)
        o = (o / l).astype(jnp.bfloat16)
        o2 = jnp.concatenate([o[r * sq:(r + 1) * sq] for r in range(rep)], axis=1)
        acc_ref[...] += jnp.dot(o2, wo_ref[pl.ds(col, gw), :], preferred_element_type=jnp.float32)

    @pl.when(g == pl.num_programs(1) - 1)
    def _():
        o_ref[0] = acc_ref[...].astype(o_ref.dtype)


@jax.jit
def pallas_standalone__gqa_block_cached__near_ridge_kernel(
    x: jax.Array,
    k_cache: jax.Array,
    v_cache: jax.Array,
    wq: jax.Array,
    wo: jax.Array,
):
    B, Sq, D = x.shape
    _, Hkv, Sk, Dh = k_cache.shape
    Hq = wq.shape[1] // Dh
    rep = Hq // Hkv
    hb = 4
    kernel = functools.partial(_gqa_kernel, hb=hb, rep=rep, dh=Dh, scale=float(Dh) ** -0.5)
    return pl.pallas_call(
        kernel,
        grid=(B, Hkv // hb),
        in_specs=[
            pl.BlockSpec((1, Sq, D), lambda b, g: (b, 0, 0)),
            pl.BlockSpec((1, hb, Sk, Dh), lambda b, g: (b, g, 0, 0)),
            pl.BlockSpec((1, hb, Sk, Dh), lambda b, g: (b, g, 0, 0)),
            pl.BlockSpec((D, Hq * Dh), lambda b, g: (0, 0)),
            pl.BlockSpec((Hq * Dh, D), lambda b, g: (0, 0)),
        ],
        out_specs=pl.BlockSpec((1, Sq, D), lambda b, g: (b, 0, 0)),
        out_shape=jax.ShapeDtypeStruct((B, Sq, D), x.dtype),
        scratch_shapes=[pltpu.VMEM((Sq, D), jnp.float32)],
        compiler_params=pltpu.CompilerParams(
            dimension_semantics=("arbitrary", "arbitrary"),
            vmem_limit_bytes=100 * 1024 * 1024,
        ),
    )(x, k_cache, v_cache, wq, wo)
```

```python
import functools

import jax
import jax.numpy as jnp
import jax.experimental.pallas as pl
import jax.experimental.pallas.tpu as pltpu

HB = 8
_NT = (((1,), (1,)), ((), ()))

def _gqa_kernel(xt_ref, k_ref, v_ref, wq_ref, wot_ref, ot_ref, x_ref, acc_ref, *, hb, rep, dh, scale):
    g = pl.program_id(1)
    sq = xt_ref.shape[2]
    gw = rep * dh

    @pl.when(g == 0)
    def _():
        acc_ref[...] = jnp.zeros(acc_ref.shape, acc_ref.dtype)
        x_ref[...] = xt_ref[0].astype(jnp.float32).T.astype(x_ref.dtype)


    x = x_ref[...]
    col0 = pl.multiple_of(g * hb * gw, hb * gw)
    q_all = jnp.dot(x, wq_ref[:, pl.ds(col0, hb * gw)], preferred_element_type=jnp.float32).astype(jnp.bfloat16)

    outs = []
    for j in range(hb):
        q2 = jnp.concatenate([q_all[:, (j * rep + r) * dh:(j * rep + r + 1) * dh] for r in range(rep)], axis=0)
        s = jax.lax.dot_general(q2, k_ref[0, j], _NT, preferred_element_type=jnp.float32) * scale
        m = jnp.max(s, axis=-1, keepdims=True)
        p = jnp.exp(s - m)
        l = jnp.sum(p, axis=-1, keepdims=True)
        o = jnp.dot(p.astype(jnp.bfloat16), v_ref[0, j], preferred_element_type=jnp.float32)
        o = (o / l).astype(jnp.bfloat16)
        outs += [o[r * sq:(r + 1) * sq] for r in range(rep)]
    o_all = jnp.concatenate(outs, axis=1)
    acc_ref[...] += jax.lax.dot_general(wot_ref[:, pl.ds(col0, hb * gw)], o_all, _NT,
                                        preferred_element_type=jnp.float32)

    @pl.when(g == pl.num_programs(1) - 1)
    def _():
        ot_ref[0] = acc_ref[...].astype(ot_ref.dtype)


@jax.jit
def pallas_standalone__gqa_block_cached__near_ridge_kernel(
    x: jax.Array,
    k_cache: jax.Array,
    v_cache: jax.Array,
    wq: jax.Array,
    wo: jax.Array,
):
    B, Sq, D = x.shape
    _, Hkv, Sk, Dh = k_cache.shape
    Hq = wq.shape[1] // Dh
    rep = Hq // Hkv
    hb = HB
    kernel = functools.partial(_gqa_kernel, hb=hb, rep=rep, dh=Dh, scale=float(Dh) ** -0.5)
    out_t = pl.pallas_call(
        kernel,
        grid=(B, Hkv // hb),
        in_specs=[
            pl.BlockSpec((1, D, Sq), lambda b, g: (b, 0, 0)),
            pl.BlockSpec((1, hb, Sk, Dh), lambda b, g: (b, g, 0, 0)),
            pl.BlockSpec((1, hb, Sk, Dh), lambda b, g: (b, g, 0, 0)),
            pl.BlockSpec((D, Hq * Dh), lambda b, g: (0, 0)),
            pl.BlockSpec((D, Hq * Dh), lambda b, g: (0, 0)),
        ],
        out_specs=pl.BlockSpec((1, D, Sq), lambda b, g: (b, 0, 0)),
        out_shape=jax.ShapeDtypeStruct((B, D, Sq), x.dtype),
        scratch_shapes=[pltpu.VMEM((Sq, D), jnp.bfloat16), pltpu.VMEM((D, Sq), jnp.float32)],
        compiler_params=pltpu.CompilerParams(
            dimension_semantics=("arbitrary", "arbitrary"),
            vmem_limit_bytes=100 * 1024 * 1024,
        ),
    )(x.transpose(0, 2, 1), k_cache, v_cache, wq, wo.T)
    return out_t.transpose(0, 2, 1)
```

```python
import functools

import jax
import jax.numpy as jnp
import jax.experimental.pallas as pl
import jax.experimental.pallas.tpu as pltpu

HB = 8
_NT = (((1,), (1,)), ((), ()))


def _gqa_kernel(xt_ref, k_ref, v_ref, wq_hbm, wot_hbm, ot_ref, x_ref, acc_ref, wq_ref, wot_ref, sems,
                *, hb, rep, dh, scale):
    b = pl.program_id(0)
    g = pl.program_id(1)
    ng = wq_ref.shape[0]
    sq = xt_ref.shape[2]
    w = hb * rep * dh

    def weight_copies(i):
        return (pltpu.make_async_copy(wq_hbm.at[:, pl.ds(i * w, w)], wq_ref.at[i], sems.at[0, i]),
                pltpu.make_async_copy(wot_hbm.at[:, pl.ds(i * w, w)], wot_ref.at[i], sems.at[1, i]))

    @pl.when(jnp.logical_and(b == 0, g == 0))
    def _():
        for i in range(ng):
            for c in weight_copies(i):
                c.start()

    @pl.when(g == 0)
    def _():
        acc_ref[...] = jnp.zeros(acc_ref.shape, acc_ref.dtype)
        x_ref[...] = xt_ref[0].astype(jnp.float32).T.astype(x_ref.dtype)

    @pl.when(b == 0)
    def _():
        for c in weight_copies(g):
            c.wait()

    q_all = jnp.dot(x_ref[...], wq_ref[g], preferred_element_type=jnp.float32).astype(jnp.bfloat16)
    outs = []
    for j in range(hb):
        q2 = jnp.concatenate([q_all[:, (j * rep + r) * dh:(j * rep + r + 1) * dh] for r in range(rep)], axis=0)
        s = jax.lax.dot_general(q2, k_ref[0, j], _NT, preferred_element_type=jnp.float32) * scale
        m = jnp.max(s, axis=-1, keepdims=True)
        p = jnp.exp(s - m)
        l = jnp.sum(p, axis=-1, keepdims=True)
        o = jnp.dot(p.astype(jnp.bfloat16), v_ref[0, j], preferred_element_type=jnp.float32)
        o = (o / l).astype(jnp.bfloat16)
        outs += [o[r * sq:(r + 1) * sq] for r in range(rep)]
    o_all = jnp.concatenate(outs, axis=1)
    acc_ref[...] += jax.lax.dot_general(wot_ref[g], o_all, _NT, preferred_element_type=jnp.float32)

    @pl.when(g == ng - 1)
    def _():
        ot_ref[0] = acc_ref[...].astype(ot_ref.dtype)


@jax.jit
def pallas_standalone__gqa_block_cached__near_ridge_kernel(
    x: jax.Array,
    k_cache: jax.Array,
    v_cache: jax.Array,
    wq: jax.Array,
    wo: jax.Array,
):
    B, Sq, D = x.shape
    _, Hkv, Sk, Dh = k_cache.shape
    Hq = wq.shape[1] // Dh
    rep = Hq // Hkv
    hb = HB
    ng = Hkv // hb
    w = hb * rep * Dh
    kernel = functools.partial(_gqa_kernel, hb=hb, rep=rep, dh=Dh, scale=float(Dh) ** -0.5)
    out_t = pl.pallas_call(
        kernel,
        grid=(B, ng),
        in_specs=[
            pl.BlockSpec((1, D, Sq), lambda b, g: (b, 0, 0)),
            pl.BlockSpec((1, hb, Sk, Dh), lambda b, g: (b, g, 0, 0)),
            pl.BlockSpec((1, hb, Sk, Dh), lambda b, g: (b, g, 0, 0)),
            pl.BlockSpec(memory_space=pl.ANY),
            pl.BlockSpec(memory_space=pl.ANY),
        ],
        out_specs=pl.BlockSpec((1, D, Sq), lambda b, g: (b, 0, 0)),
        out_shape=jax.ShapeDtypeStruct((B, D, Sq), x.dtype),
        scratch_shapes=[
            pltpu.VMEM((Sq, D), jnp.bfloat16),
            pltpu.VMEM((D, Sq), jnp.float32),
            pltpu.VMEM((ng, D, w), jnp.bfloat16),
            pltpu.VMEM((ng, D, w), jnp.bfloat16),
            pltpu.SemaphoreType.DMA((2, ng)),
        ],
        compiler_params=pltpu.CompilerParams(
            dimension_semantics=("arbitrary", "arbitrary"),
            vmem_limit_bytes=100 * 1024 * 1024,
        ),
    )(x.transpose(0, 2, 1), k_cache, v_cache, wq, wo.T)
    return out_t.transpose(0, 2, 1)
```
